```python
import os as _os
_os.environ.setdefault("JAX_PLATFORMS", "cpu")
import jax
import jax.numpy as jnp

def _softmax(x, axis=-1):
    return jax.nn.softmax(x, axis=axis)
def _gelu(x):
    return jax.nn.gelu(x, approximate=True)
def _silu(x):
    return jax.nn.silu(x)
def _sigmoid(x):
    return jax.nn.sigmoid(x)
def _layernorm(x, axis=-1, eps=1e-5):
    m = jnp.mean(x, axis=axis, keepdims=True)
    v = jnp.var(x, axis=axis, keepdims=True)
    return (x - m) / jnp.sqrt(v + eps)
def _scatter_add(tgt, idx, src, axis=0):
    return tgt.at[idx].add(src)
def _segment_sum(src, seg, n):
    return jax.ops.segment_sum(src, seg, n)
class _Rng:
    def __init__(self, key):
        self._k = key
    def _next(self):
        self._k, sub = jax.random.split(self._k)
        return sub
    def normal(self, shape):
        return jax.random.normal(self._next(), shape, dtype=jnp.bfloat16)
    def randint(self, lo, hi, shape):
        return jax.random.randint(self._next(), shape, lo, hi, dtype=jnp.int32)
    def uniform(self, shape, lo=0.0, hi=1.0):
        return jax.random.uniform(self._next(), shape, jnp.bfloat16, lo, hi)
    def permutation(self, n):
        return jax.random.permutation(self._next(), n)


kernel_name = 'concat_heads__linear_attn_block__sliding_local_dilated__prompt'

def setup_inputs():
    _rng = _Rng(jax.random.key(int.from_bytes(__import__("os").urandom(4), "little")))
    _w = (lambda a: (lambda t: t.astype(jnp.bfloat16) if jnp.issubdtype(t.dtype, jnp.floating) else t)(jnp.asarray(a)))
    def _A_setup():
        B, S, D = 1, 2048, 576
        return {
            "x": _w((lambda *s: _rng.normal(s) * 0.05)(B, S, D)),
            "wqkv": _w((lambda *s: _rng.normal(s) * 1.6)(D, 3 * D)),
            "wo": _w((lambda *s: _rng.normal(s) * 0.4)(D, D)),
        }
    _A_in = _A_setup()

    def _B_setup():
        B, S, D = 1, 2048, 576
        return {
            "x": _w((lambda *s: _rng.normal(s) * 0.2)(B, S, D)),
            "wqkv": _w((lambda *s: _rng.normal(s) * 0.2)(D, 3 * D)),
            "wo": _w((lambda *s: _rng.normal(s) * 0.05)(D, D)),
        }
    _B_in = _B_setup()

    return {
        "A_x": _A_in["x"],
        "A_wqkv": _A_in["wqkv"],
        "A_wo": _A_in["wo"],
        "B_x": _B_in["x"],
        "B_wqkv": _B_in["wqkv"],
        "B_wo": _B_in["wo"],
    }

def reference(A_x, A_wqkv, A_wo, B_x, B_wqkv, B_wo):
    def _A_ref(x, wqkv, wo):
        B, S, D = x.shape
        H = 32; Dh = D // H
        qkv = (lambda x, *d: x.transpose(*d))((x @ wqkv).reshape(B, S, 3, H, Dh), 2, 0, 3, 1, 4)
        q, k, v = qkv[0], qkv[1], qkv[2]
        phi = lambda t: jnp.where(t > 0, t + 1, jnp.exp(t)) + 1e-6
        pq, pk = phi(q), phi(k)
        kv = jnp.einsum("bhsd,bhse->bhde", pk, v)
        z = jnp.einsum("bhsd->bhd", pk)
        num = jnp.einsum("bhqd,bhde->bhqe", pq, kv)
        den = jnp.einsum("bhqd,bhd->bhq", pq, z)[..., None] + 1e-6
        o = num / den
        return (lambda x, *d: x.transpose(*d))(o, 0, 2, 1, 3).reshape(B, S, D) @ wo

    def _B_ref(x, wqkv, wo):
        B, S, D = x.shape
        H = 32; Dh = D // H
        W, dil = 8, 2
        qkv = (lambda x, *d: x.transpose(*d))((x @ wqkv).reshape(B, S, 3, H, Dh), 2, 0, 3, 1, 4)
        q, k, v = qkv[0], qkv[1], qkv[2]
        scale = Dh ** -0.5
        pos = jnp.arange(S)
        off = jnp.arange(W) * dil
        idx = pos[:, None] - off[None, :]
        mask = idx >= 0
        idx_c = jnp.where(mask, idx, 0).reshape(-1)
        kg = k[:, :, idx_c, :].reshape(B, H, S, W, Dh)
        vg = v[:, :, idx_c, :].reshape(B, H, S, W, Dh)
        logits = jnp.einsum("bhsd,bhswd->bhsw", q, kg) * scale
        logits = jnp.where(mask[None, None, :, :], logits, -1e9)
        attn = _softmax(logits, axis=-1)
        o = jnp.einsum("bhsw,bhswd->bhsd", attn, vg)
        return (lambda x, *d: x.transpose(*d))(o, 0, 2, 1, 3).reshape(B, S, D) @ wo

    a = _A_ref(A_x, A_wqkv, A_wo)
    b = _B_ref(B_x, B_wqkv, B_wo)
    return jnp.concatenate([a, b], axis=-1)
```

```python
import contextlib
import functools
import jax
import jax.numpy as jnp
import jax.experimental.pallas as pl
import jax.experimental.pallas.tpu as pltpu

S = 2048
D = 576
H = 32
DH = 18
W = 8
DIL = 2
BF = jnp.bfloat16
F32 = jnp.float32
U32 = jnp.uint32
NT = S // 128
CT = 5
NG = 4
GR = 144


def _cw(ct):
    return min(128, D - ct * 128)


def build(scopes=False, qpack=False, p2='a', otb=1, p1='a'):
    def scope(name):
        return jax.named_scope(name) if scopes else contextlib.nullcontext()

    def kernel(xa_hbm, wa_hbm, woa_hbm, xb_hbm, wb_hbm, wob_hbm, out_hbm,
               xa_v, xb_v, wa_v, wb_v, woa_v, wob_v, t32a, t32b, t32o,
               wqa, wka, wbT, wobT, m32, mT, zb, qB, kB, vB, obuf,
               sem_x, sem_w, sem_o):
        def xcopy(src, dst, t, si):
            return pltpu.make_async_copy(
                src.at[:, pl.ds(t * 128, 128)], dst.at[t], sem_x.at[si])

        def wcol(src, dst, c0, c1, si):
            return pltpu.make_async_copy(
                src.at[:, pl.ds(c0, c1 - c0)], dst.at[:, pl.ds(c0, c1 - c0)],
                sem_w.at[si])

        c_wk = wcol(wa_hbm, wa_v, 512, 1152, 0)
        c_wq = wcol(wa_hbm, wa_v, 0, 512, 1)
        c_wv = wcol(wa_hbm, wa_v, 1152, 1728, 2)
        c_wb = pltpu.make_async_copy(wb_hbm, wb_v, sem_w.at[3])
        c_woa = pltpu.make_async_copy(woa_hbm, woa_v, sem_w.at[4])
        c_wob = pltpu.make_async_copy(wob_hbm, wob_v, sem_w.at[5])
        cxa = [xcopy(xa_hbm, xa_v, t, t) for t in range(NT)]
        cxb = [xcopy(xb_hbm, xb_v, t, NT + t) for t in range(NT)]

        def transpose_tiles(w_v, t32, n_lo, n_hi):
            for n0 in range(n_lo, n_hi, 128):
                n1 = min(n0 + 128, n_hi)
                for ct in range(CT):
                    cw = _cw(ct)
                    blk = w_v[ct * 128:ct * 128 + cw, n0:n1].astype(F32)
                    t32[ct, n0:n1, 0:cw] = blk.T

        def gather_perm(dst, dst_row0, t32, src_row0):
            for g in range(NG):
                for d2 in range(DH // 2):
                    for ct in range(CT):
                        lo = t32[ct, pl.ds(src_row0 + g * GR + 2 * d2, 8, stride=DH), :]
                        hi = t32[ct, pl.ds(src_row0 + g * GR + 2 * d2 + 1, 8, stride=DH), :]
                        rows = jnp.concatenate([lo, hi], axis=0)
                        r = dst_row0 + g * GR + d2 * 16
                        dst[ct, r:r + 16, :] = rows.astype(BF)

        def ld(ref_u32_slab):
            return pltpu.bitcast(ref_u32_slab, BF)

        def lhs(ref):
            u = ref.bitcast(U32)
            return jnp.concatenate([ld(u[c]) for c in range(CT)], axis=1)[:, :D]

        def xt(ref, t):
            return ld(ref.bitcast(U32)[t])

        def phi(t):
            return jnp.where(t > 0, t + 1.0, jnp.exp(t)) + 1e-6

        def prep_wob():
            for ct in range(CT):
                cw = _cw(ct)
                t32o[ct, :, 0:cw] = wob_v[:, ct * 128:ct * 128 + cw].astype(F32)
            for ct in range(CT):
                cw = _cw(ct)
                parts = []
                for g in range(NG):
                    for e in range(DH):
                        parts.append(t32o[ct, pl.ds(g * GR + e, 8, stride=DH), :])
                full = jnp.concatenate(parts, axis=0)
                for rt in range(CT):
                    rw = _cw(rt)
                    wobT[rt, ct * 128:ct * 128 + cw, 0:rw] = (
                        full[rt * 128:rt * 128 + rw, :].T[0:cw, :].astype(BF))

        lane = jax.lax.broadcasted_iota(jnp.int32, (1, 128), 1)
        st = {}

        def k_tile(t):
            pk = phi(jnp.dot(lhs(wka), xt(xa_v, t), preferred_element_type=F32))
            st['z'] = pk if 'z' not in st else st['z'] + pk
            st[('pk', t)] = pk.astype(BF)

        def g_block(b):
            pk = jnp.concatenate([st.pop(('pk', t)) for t in range(4 * b, 4 * b + 4)], axis=1)
            xblk = jnp.concatenate([xt(xa_v, t) for t in range(4 * b, 4 * b + 4)], axis=1)
            gt = jax.lax.dot_general(pk, xblk, (((1,), (1,)), ((), ())),
                                     preferred_element_type=F32)
            st['g'] = gt if 'g' not in st else st['g'] + gt

        def small_kv():
            z = jnp.sum(st['z'], axis=1, keepdims=True)
            zb[...] = jnp.broadcast_to(z, (D, 128))
            gb = st['g'].astype(BF)
            for g in range(NG):
                n0 = 128 * g
                n1 = min(n0 + 256, D)
                kv = jnp.dot(gb[g * GR:(g + 1) * GR, :], wa_v[:, 2 * D + n0:2 * D + n1],
                             preferred_element_type=F32)
                row = jax.lax.broadcasted_iota(jnp.int32, kv.shape, 0)
                col = jax.lax.broadcasted_iota(jnp.int32, kv.shape, 1) + n0
                same = ((col * 3641) >> 16) == (row & 7) + 8 * g
                st[('kv', g)] = jnp.where(same, kv, 0.0).astype(BF)

        def small_m():
            for g in range(NG):
                n0 = 128 * g
                n1 = min(n0 + 256, D)
                m32[g * GR:(g + 1) * GR, :] = jnp.dot(
                    st.pop(('kv', g)), woa_v[n0:n1, :], preferred_element_type=F32)

        def small_t():
            for rt in range(CT):
                rw = _cw(rt)
                for ct in range(CT):
                    cw = _cw(ct)
                    mT[rt, ct * 128:ct * 128 + cw, 0:rw] = (
                        m32[rt * 128:rt * 128 + rw, ct * 128:ct * 128 + cw].T.astype(BF))

        def qkv_tile(t):
            qkv = jnp.dot(lhs(wbT), xt(xb_v, t), preferred_element_type=F32)
            if qpack:
                qB[t] = qkv[0:D].astype(BF)
            else:
                st[('q', t)] = qkv[0:D]
            kB[t + 1] = qkv[D:2 * D].astype(BF)
            vB[t + 1] = qkv[2 * D:3 * D].astype(BF)

        def unpack(u):
            return pltpu.bitcast(u, BF).astype(F32)

        def shifted(prev, cur, w):
            if w == 0:
                return cur
            return pltpu.roll(jnp.where(lane >= 128 - DIL * w, prev, cur), DIL * w, axis=1)

        def attn_tile(t):
            ku = kB.bitcast(U32)
            vu = vB.bitcast(U32)
            o_parts = []
            for g in range(NG):
                r0 = g * (GR // 2)
                r1 = r0 + GR // 2
                if qpack:
                    q3 = unpack(qB.bitcast(U32)[t, r0:r1, :]).reshape(DH, 8, 128)
                else:
                    q3 = st[('q', t)][g * GR:(g + 1) * GR].reshape(DH, 8, 128)
                kc = ku[t + 1, r0:r1, :]
                kp = ku[t, r0:r1, :]
                logits = []
                for w in range(W):
                    ks = unpack(shifted(kp, kc, w)).reshape(DH, 8, 128)
                    lw = jnp.sum(q3 * ks, axis=0) * (DH ** -0.5)
                    if t == 0 and w > 0:
                        lw = jnp.where(lane >= DIL * w, lw, -1e9)
                    logits.append(lw)
                m = functools.reduce(jnp.maximum, logits)
                es = [jnp.exp(l - m) for l in logits]
                rs = 1.0 / functools.reduce(jnp.add, es)
                vc = vu[t + 1, r0:r1, :]
                vp = vu[t, r0:r1, :]
                o = None
                for w in range(W):
                    vs = unpack(shifted(vp, vc, w)).reshape(DH, 8, 128)
                    c = vs * (es[w] * rs)[None]
                    o = c if o is None else o + c
                o_parts.append(o.reshape(GR, 128))
            if not qpack:
                del st[('q', t)]
            st[('o', t)] = jnp.concatenate(o_parts, axis=0).astype(BF)

        def qa_tile(t):
            pj = phi(jnp.dot(lhs(wqa), xt(xa_v, t), preferred_element_type=F32))
            tt = (pj * zb[...]).reshape(NG, DH, 8, 128)
            den = jnp.sum(tt, axis=1, keepdims=True) + 1e-6
            pn = pj.reshape(NG, DH, 8, 128) * (1.0 / den)
            st[('pqn', t)] = pn.reshape(D, 128).astype(BF)

        def outb_tile(t):
            st[('outb', t)] = jnp.dot(lhs(wobT), st.pop(('o', t)), preferred_element_type=F32)

        def outa_tile(t):
            st[('outa', t)] = jnp.dot(lhs(mT), st.pop(('pqn', t)), preferred_element_type=F32)

        ocopies = []

        def store_tile(t):
            full = jnp.concatenate([st.pop(('outa', t)), st.pop(('outb', t))], axis=0).astype(BF)
            obuf[t] = full.T
            if (t + 1) % otb == 0:
                b = t // otb
                for u in range(otb):
                    tu = b * otb + u
                    c = pltpu.make_async_copy(
                        obuf.at[tu], out_hbm.at[pl.ds(tu * 128, 128), :], sem_o.at[tu])
                    c.start()
                    ocopies.append(c)

        def start(cs):
            for c in cs:
                c.start()

        def wait(cs):
            for c in cs:
                c.wait()

        start([c_wk] + cxa[0:4])
        with scope("pro0"):
            c_wk.wait()
            start(cxa[4:8] + [c_wb])
            transpose_tiles(wa_v, t32a, 512, 1152)
            gather_perm(wka, 0, t32a, D)
            wait(cxa[0:4])
        with scope("p1a"):
            start(cxa[8:12] + [c_wq])
            k_tile(0)
            kB[0] = jnp.zeros((D, 128), BF)
            vB[0] = jnp.zeros((D, 128), BF)
            for t in range(1, 4):
                k_tile(t)
            wait(cxa[4:8])
            start(cxa[12:16] + [c_wob, c_wv, c_woa])
            k_tile(4)
            k_tile(5)
            g_block(0)
            wait([c_wb] + cxa[8:12] + [c_wq])
            start(cxb)
            k_tile(6)
            k_tile(7)
            transpose_tiles(wb_v, t32b, 0, 640)
            k_tile(8)
            k_tile(9)
            gather_perm(wbT, 0, t32b, 0)
        with scope("p1b"):
            wait(cxa[12:16] + [c_wob, c_wv, c_woa])
            g_block(1)
            transpose_tiles(wb_v, t32b, 640, 1152)
            gather_perm(wbT, D, t32b, D)
            k_tile(10)
            k_tile(11)
            transpose_tiles(wb_v, t32b, 1152, 1728)
            k_tile(12)
            k_tile(13)
            gather_perm(wbT, 2 * D, t32b, 2 * D)
            g_block(2)
            transpose_tiles(wa_v, t32a, 0, 512)
            gather_perm(wqa, 0, t32a, 0)
            k_tile(14)
            k_tile(15)
            wait(cxb)
            qkv_tile(0)
            prep_wob()
            g_block(3)
        with scope("mid"):
            qkv_tile(1)
            small_kv()
            small_m()
            small_t()
        if p2 == 'a':
            DL = 2
            for t in range(NT):
                with scope(f"p2_{t // 4}"):
                    if t + DL < NT:
                        qkv_tile(t + DL)
                    qa_tile(t)
                    attn_tile(t)
                    outb_tile(t)
                    outa_tile(t)
                    store_tile(t)
        elif p2 == 'b':
            DL = 2
            for t in range(NT + 1):
                with scope(f"p2_{t // 4}"):
                    if t + DL < NT:
                        qkv_tile(t + DL)
                    if t < NT:
                        attn_tile(t)
                        qa_tile(t)
                    if t > 0:
                        outb_tile(t - 1)
                        outa_tile(t - 1)
                        store_tile(t - 1)
        elif p2 == 'c':
            DL = 2
            for t in range(NT + 1):
                with scope(f"p2_{t // 4}"):
                    if t > 0:
                        outb_tile(t - 1)
                        outa_tile(t - 1)
                        store_tile(t - 1)
                    if t < NT:
                        qa_tile(t)
                        attn_tile(t)
                    if t + DL < NT:
                        qkv_tile(t + DL)
        for c in ocopies:
            c.wait()

    scratch = [
        pltpu.VMEM((NT, D, 128), BF),
        pltpu.VMEM((NT, D, 128), BF),
        pltpu.VMEM((D, 3 * D), BF),
        pltpu.VMEM((D, 3 * D), BF),
        pltpu.VMEM((D, D), BF),
        pltpu.VMEM((D, D), BF),
        pltpu.VMEM((CT, 2 * D, 128), F32),
        pltpu.VMEM((CT, 3 * D, 128), F32),
        pltpu.VMEM((CT, D, 128), F32),
        pltpu.VMEM((CT, D, 128), BF),
        pltpu.VMEM((CT, D, 128), BF),
        pltpu.VMEM((CT, 3 * D, 128), BF),
        pltpu.VMEM((CT, D, 128), BF),
        pltpu.VMEM((D, D), F32),
        pltpu.VMEM((CT, D, 128), BF),
        pltpu.VMEM((D, 128), F32),
        pltpu.VMEM((NT, D, 128), BF),
        pltpu.VMEM((NT + 1, D, 128), BF),
        pltpu.VMEM((NT + 1, D, 128), BF),
        pltpu.VMEM((NT, 128, 2 * D), BF),
        pltpu.SemaphoreType.DMA((2 * NT,)),
        pltpu.SemaphoreType.DMA((6,)),
        pltpu.SemaphoreType.DMA((NT,)),
    ]

    def f(A_x, A_wqkv, A_wo, B_x, B_wqkv, B_wo):
        out = pl.pallas_call(
            kernel,
            out_shape=jax.ShapeDtypeStruct((S, 2 * D), BF),
            in_specs=[pl.BlockSpec(memory_space=pl.ANY)] * 6,
            out_specs=pl.BlockSpec(memory_space=pl.ANY),
            scratch_shapes=scratch,
            compiler_params=pltpu.CompilerParams(vmem_limit_bytes=110 * 2**20),
        )(A_x[0].T, A_wqkv, A_wo, B_x[0].T, B_wqkv, B_wo)
        return out[None]
    f.__name__ = 'kern'
    return jax.jit(f)


_impl = build()


@jax.jit
def pallas_concat_heads__linear_attn_block__sliding_local_dilated__prompt_kernel(
    A_x: jax.Array,
    A_wqkv: jax.Array,
    A_wo: jax.Array,
    B_x: jax.Array,
    B_wqkv: jax.Array,
    B_wo: jax.Array,
):
    return _impl(A_x, A_wqkv, A_wo, B_x, B_wqkv, B_wo)
```

```python
import contextlib
import functools
import jax
import jax.numpy as jnp
import jax.experimental.pallas as pl
import jax.experimental.pallas.tpu as pltpu

S = 2048
D = 576
H = 32
DH = 18
W = 8
DIL = 2
BF = jnp.bfloat16
F32 = jnp.float32
U32 = jnp.uint32
NT = S // 128
CT = 5
NG = 4
GR = 144


def _cw(ct):
    return min(128, D - ct * 128)


def build(scopes=False, qpack=False, p2='a', otb=1, p1='a', kf32=False, flags=None, pin='grid', KH=0, mw=True, wobpos=0, split=False, wqpos=0, DC=18, dbg='', DLA=2, order='QATBOS'):
    def scope(name):
        on = scopes and (scopes is True or name.startswith('wait'))
        return jax.named_scope(name) if on else contextlib.nullcontext()

    def kernel(xa_hbm, wa_hbm, woa_hbm, xb_hbm, wb_hbm, wob_hbm, out_hbm,
               xa_v, xb_v, wa_v, wb_v, woa_v, wob_v, t32a, t32b, tbo,
               wqa, wka, wbT, wobT, m32, mT, zb, pkb, kB, vB, obuf,
               sem_x, sem_w, sem_o):
        def xcopy(src, dst, t, si):
            return pltpu.make_async_copy(
                src.at[:, pl.ds(pl.multiple_of(t * 128, 128), 128)], dst.at[t], sem_x.at[si])

        def colcopy(src, dst, c, si):
            c0 = pl.multiple_of(c * 128, 128)
            return pltpu.make_async_copy(
                src.at[:, pl.ds(c0, 128)], dst.at[:, pl.ds(c0, 128)], sem_w.at[si])

        def rowcopy(src, dst, i, c0, nc, si):
            r0 = pl.multiple_of(i * (D // 2), D // 2)
            return pltpu.make_async_copy(
                src.at[pl.ds(r0, D // 2), pl.ds(c0, nc)],
                dst.at[pl.ds(r0, D // 2), pl.ds(c0, nc)], sem_w.at[si])

        d_wk = (5, lambda i: colcopy(wa_hbm, wa_v, 4 + i, i))
        d_xa0 = (12, lambda i: xcopy(xa_hbm, xa_v, i, i))
        d_xa1 = (4, lambda i: xcopy(xa_hbm, xa_v, 12 + i, 12 + i))
        d_wb = (2, lambda i: rowcopy(wb_hbm, wb_v, i, 0, 3 * D, 5 + i))
        d_wq = (2, lambda i: rowcopy(wa_hbm, wa_v, i, 0, 512, 7 + i))
        d_xb0 = (2, lambda i: xcopy(xb_hbm, xb_v, i, NT + i))
        d_wv = (2, lambda i: rowcopy(wa_hbm, wa_v, i, 2 * D, D, 9 + i))
        d_woa = (2, lambda i: rowcopy(woa_hbm, woa_v, i, 0, D, 11 + i))
        d_wob = (2, lambda i: rowcopy(wob_hbm, wob_v, i, 0, D, 13 + i))
        d_xb1 = (NT - 2, lambda i: xcopy(xb_hbm, xb_v, 2 + i, NT + 2 + i))

        def issue(dsc):
            n, mk = dsc

            def body(i, c):
                mk(i).start()
                return c
            jax.lax.fori_loop(0, n, body, 0)

        def every(dsc):
            return [dsc[1](i) for i in range(dsc[0])]

        cwk = every(d_wk)
        cxa = every(d_xa0) + every(d_xa1)
        cxb = every(d_xb0) + every(d_xb1)
        c_wb, c_wq, c_wv, c_woa, c_wob = (every(x) for x in (d_wb, d_wq, d_wv, d_woa, d_wob))

        zero = pl.program_id(0) if pin == 'grid' else 0
        sub = jax.lax.broadcasted_iota(jnp.int32, (8, 128), 0)

        def transpose_tiles(w_v, tb, n_lo, n_hi):
            for n0 in range(n_lo, n_hi, 128):
                n1 = min(n0 + 128, n_hi)
                for ct in range(CT):
                    cw = _cw(ct)
                    tb.bitcast(U32)[ct, n0 // 2:n1 // 2, 0:cw] = pltpu.bitcast(
                        w_v[ct * 128:ct * 128 + cw, n0:n1].T, U32)

        def perm_rows(load, row0, pairs=(0, 2)):
            out = [None] * (NG * (DH // 2))
            for g in pairs:
                for d2 in range(DH // 2):
                    base = row0 // 2 + g * (GR // 2) + d2
                    ev = load(base)
                    od = load(base + DH // 2)
                    p = (ev & jnp.uint32(0xFFFF)) | (od << 16)
                    q = (ev >> 16) | (od & jnp.uint32(0xFFFF0000))
                    out[g * (DH // 2) + d2] = jnp.where(sub < 4, p, pltpu.roll(q, 4, axis=0))
                    out[(g + 1) * (DH // 2) + d2] = jnp.where(sub < 4, pltpu.roll(p, 4, axis=0), q)
            return jnp.concatenate([o for o in out if o is not None], axis=0)

        def gather_perm(dst, dst_row0, tb, src_row0, pairs=(0, 2)):
            tu = tb.bitcast(U32)
            for ct in range(CT):
                for g in pairs:
                    w0 = (dst_row0 + g * GR) // 2
                    dst.bitcast(U32)[ct, w0:w0 + GR, :] = perm_rows(
                        lambda r: tu[ct, pl.ds(r, 8, stride=DH), :], src_row0, (g,))

        def ld(ref_u32_slab):
            return pltpu.bitcast(ref_u32_slab, BF)

        def lhs(ref, r0=0, r1=D):
            u = ref.bitcast(U32)
            return jnp.concatenate(
                [ld(u[c, r0 // 2:r1 // 2, :]) for c in range(CT)], axis=1)[:, :D]

        def xt(ref, t):
            return ld(ref.bitcast(U32)[t])

        def phi(t):
            return jnp.where(t > 0, t + 1.0, jnp.exp(t)) + 1e-6

        def prep_wob():
            for ct in range(CT):
                cw = _cw(ct)
                tbo.bitcast(U32)[ct, :, 0:cw] = wob_v.bitcast(U32)[:, ct * 128:ct * 128 + cw]
            tu = tbo.bitcast(U32)
            for ct in range(CT):
                cw = _cw(ct)
                full = pltpu.bitcast(
                    perm_rows(lambda r: tu[ct, pl.ds(r, 8, stride=DH), :], 0), BF)
                for rt in range(CT):
                    rw = _cw(rt)
                    wobT.bitcast(U32)[rt, ct * 64:ct * 64 + cw // 2, 0:rw] = pltpu.bitcast(
                        full[rt * 128:rt * 128 + rw, 0:cw].T, U32)

        lane = jax.lax.broadcasted_iota(jnp.int32, (1, 128), 1)

        def kdot(t):
            if t < KH:
                return jnp.concatenate(
                    [jnp.dot(lhs(wka, h * D // 2, (h + 1) * D // 2), xt(xa_v, t),
                             preferred_element_type=F32) for h in range(2)], axis=0)
            return jnp.dot(lhs(wka), xt(xa_v, t), preferred_element_type=F32)
        st = {}

        def k_mm(t):
            st[('kt', t)] = kdot(t)

        def k_tile(t):
            k_mm(t)
            k_post(t)

        def k_post(t):
            pk = phi(st.pop(('kt', t)))
            st['z'] = pk if 'z' not in st else st['z'] + pk
            pkb[t] = pk.astype(BF)

        def prep_wq():
            transpose_tiles(wa_v, t32a, 0, 512)
            gather_perm(wqa, 0, t32a, 0)

        def g_block(b):
            pk = jnp.concatenate([xt(pkb, t) for t in range(4 * b, 4 * b + 4)], axis=1)
            xblk = jnp.concatenate([xt(xa_v, t) for t in range(4 * b, 4 * b + 4)], axis=1)
            gt = jax.lax.dot_general(pk, xblk, (((1,), (1,)), ((), ())),
                                     preferred_element_type=F32)
            st['g'] = gt if 'g' not in st else st['g'] + gt

        def small_kv():
            z = jnp.sum(st['z'], axis=1, keepdims=True)
            zb[...] = jnp.broadcast_to(z, (D, 128))
            gb = st['g'].astype(BF)
            for g in range(NG):
                n0 = 128 * g
                n1 = min(n0 + 256, D)
                kv = jnp.dot(gb[g * GR:(g + 1) * GR, :], wa_v[:, 2 * D + n0:2 * D + n1],
                             preferred_element_type=F32)
                row = jax.lax.broadcasted_iota(jnp.int32, kv.shape, 0)
                col = jax.lax.broadcasted_iota(jnp.int32, kv.shape, 1) + n0
                same = ((col * 3641) >> 16) == (row & 7) + 8 * g
                st[('kv', g)] = jnp.where(same, kv, 0.0).astype(BF)

        def small_m():
            for g in range(NG):
                n0 = 128 * g
                n1 = min(n0 + 256, D)
                m32[g * GR:(g + 1) * GR, :] = jnp.dot(
                    st.pop(('kv', g)), woa_v[n0:n1, :], preferred_element_type=F32).astype(BF)

        def small_t():
            for rt in range(CT):
                rw = _cw(rt)
                for ct in range(CT):
                    cw = _cw(ct)
                    mT.bitcast(U32)[rt, ct * 64:ct * 64 + cw // 2, 0:rw] = pltpu.bitcast(
                        m32[rt * 128:rt * 128 + rw, ct * 128:ct * 128 + cw].T, U32)

        def qkv_tile(t):
            if t == 2 and not mw:
                wait(cxb[2:16])
            qkv = jnp.dot(lhs(wbT, 0, 3 * D), xt(xb_v, t), preferred_element_type=F32)
            st[('q', t)] = qkv[0:D]
            kB[t + 1] = qkv[D:2 * D].astype(kB.dtype)
            vB[t + 1] = qkv[2 * D:3 * D].astype(vB.dtype)

        def unpack(u):
            return pltpu.bitcast(u, BF).astype(F32)

        def shifted(prev, cur, w):
            if w == 0:
                return cur
            return pltpu.roll(jnp.where(lane >= 128 - DIL * w, prev, cur), DIL * w, axis=1)

        def attn_tile(t):
            o_parts = []
            nd = DH // DC
            for g in range(NG):
                logits = [None] * W
                for c in range(nd):
                    r0 = g * GR + c * DC * 8
                    r1 = r0 + DC * 8
                    q3 = st[('q', t)][r0:r1].reshape(DC, 8, 128)
                    kc = kB[t + 1, r0:r1, :]
                    kp = kB[t, r0:r1, :] if t > 0 else jnp.zeros_like(kc)
                    for w in range(W):
                        ks = shifted(kp, kc, w).reshape(DC, 8, 128)
                        part = jnp.sum(q3 * ks, axis=0)
                        logits[w] = part if c == 0 else logits[w] + part
                for w in range(W):
                    lw = logits[w] * (DH ** -0.5)
                    if t == 0 and w > 0:
                        lw = jnp.where(lane >= DIL * w, lw, -1e9)
                    logits[w] = lw
                m = functools.reduce(jnp.maximum, logits)
                es = [jnp.exp(l - m) for l in logits]
                rs = 1.0 / functools.reduce(jnp.add, es)
                ps = [(e * rs)[None] for e in es]
                for c in range(nd):
                    r0 = g * GR + c * DC * 8
                    r1 = r0 + DC * 8
                    vc = vB[t + 1, r0:r1, :]
                    vp = vB[t, r0:r1, :] if t > 0 else jnp.zeros_like(vc)
                    o = None
                    for w in range(W):
                        cw = shifted(vp, vc, w).reshape(DC, 8, 128) * ps[w]
                        o = cw if o is None else o + cw
                    o_parts.append(o.reshape(DC * 8, 128))
            qq = st.pop(('q', t))
            ov = jnp.concatenate(o_parts, axis=0).astype(BF)
            if 'noattn' in dbg:
                ov = (vB[t + 1] + kB[t + 1] + qq).astype(BF)
            if pin:
                for b in range(CT):
                    obuf[NT + (t % 2) + zero, 0:_cw(b), 128 * b:128 * (b + 1)] = (
                        ov[128 * b:128 * b + _cw(b), :])
            else:
                st[('o', t)] = ov

        def qa_tile(t):
            pj = phi(jnp.dot(lhs(wqa), xt(xa_v, t), preferred_element_type=F32))
            tt = (pj * zb[...]).reshape(NG, DH, 8, 128)
            den = jnp.sum(tt, axis=1, keepdims=True) + 1e-6
            pn = pj.reshape(NG, DH, 8, 128) * (1.0 / den)
            st[('pqn', t)] = pn.reshape(D, 128).astype(BF)

        def outb_tile(t):
            if pin:
                ov = jnp.concatenate(
                    [obuf[NT + (t % 2) + zero, 0:_cw(b), 128 * b:128 * (b + 1)] for b in range(CT)],
                    axis=0)
            else:
                ov = st.pop(('o', t))
            st[('outb', t)] = jnp.dot(lhs(wobT), ov, preferred_element_type=F32)

        def outa_tile(t):
            st[('outa', t)] = jnp.dot(lhs(mT), st.pop(('pqn', t)), preferred_element_type=F32)

        ocopies = []

        def store_tile(t):
            full = jnp.concatenate([st.pop(('outa', t)), st.pop(('outb', t))], axis=0).astype(BF)
            obuf[t] = full.T
            if (t + 1) % otb == 0:
                b = t // otb
                for u in range(otb):
                    tu = b * otb + u
                    c = pltpu.make_async_copy(
                        obuf.at[tu], out_hbm.at[pl.ds(tu * 128, 128), :], sem_o.at[tu])
                    if 'nodma' in dbg and tu != NT - 1:
                        continue
                    c.start()
                    ocopies.append(c)

        done = set()

        def wait(cs):
            done.add(len(done))
            with scope(f"wait{len(done)}"):
                for c in cs:
                    c.wait()

        for dsc in (d_wk, d_xa0, d_wb, d_xa1, d_wq, d_xb0, d_wv, d_woa, d_wob, d_xb1):
            issue(dsc)
        with scope("pro0"):
            for i in range(3):
                wait([cwk[i]])
                transpose_tiles(wa_v, t32a, 512 + 128 * i, 640 + 128 * i)
            gather_perm(wka, 0, t32a, D, (0,))
            for i in range(3, 5):
                wait([cwk[i]])
                transpose_tiles(wa_v, t32a, 512 + 128 * i, 640 + 128 * i)
            gather_perm(wka, 0, t32a, D, (2,))
            wait(cxa[0:2])
        with scope("p1a"):
            if split:
                k_mm(0)
                k_mm(1)
                k_post(0)
                wait(cxa[2:4])
                k_mm(2)
                k_post(1)
                k_mm(3)
                k_post(2)
                wait(cxa[4:12])
                k_mm(4)
                k_post(3)
                for t in range(5, 8):
                    k_mm(t)
                    k_post(t - 1)
                g_block(0)
                k_post(7)
                for t in range(8, 12):
                    k_mm(t)
                    if t > 8:
                        k_post(t - 1)
            else:
                k_tile(0)
                k_tile(1)
                wait(cxa[2:4])
                k_tile(2)
                k_tile(3)
                wait(cxa[4:12])
                for t in range(4, 8):
                    k_tile(t)
                g_block(0)
                for t in range(8, 12):
                    k_tile(t)
        with scope("p1b"):
            wait(cxa[12:16] + c_wb)
            transpose_tiles(wb_v, t32b, 0, 640)
            if split:
                k_post(11)
            g_block(1)
            gather_perm(wbT, 0, t32b, 0)
            transpose_tiles(wb_v, t32b, 640, 1152)
            for t in range(12, 16):
                k_tile(t)
            gather_perm(wbT, D, t32b, D)
            transpose_tiles(wb_v, t32b, 1152, 1728)
            gather_perm(wbT, 2 * D, t32b, 2 * D)
            g_block(2)
        with scope("mid"):
            wait(c_wq + cxb[0:2] + c_wv + c_woa + c_wob + (cxb[2:16] if mw else []))
            qkv_tile(0)
            if wqpos == 0:
                prep_wq()
            g_block(3)
            if wqpos == 2:
                prep_wq()
            if DLA > 1:
                qkv_tile(1)
            if wqpos == 1:
                prep_wq()
            if wobpos == 0:
                prep_wob()
            small_kv()
            if wobpos == 1:
                prep_wob()
            small_m()
            if wobpos == 2:
                prep_wob()
            small_t()
            if wobpos == 3:
                prep_wob()
        if p2 == 'a':
            DL = DLA
            for t in range(2, DL):
                qkv_tile(t)
            for t in range(NT):
                for ch in order:
                    if ch == 'Q' and t + DL < NT:
                        qkv_tile(t + DL)
                    elif ch == 'A':
                        qa_tile(t)
                    elif ch == 'T':
                        attn_tile(t)
                    elif ch == 'B':
                        outb_tile(t)
                    elif ch == 'O':
                        outa_tile(t)
                    elif ch == 'S':
                        store_tile(t)
        elif p2 == 'b':
            DL = 2
            for t in range(NT + 1):
                with scope(f"p2_{t // 4}"):
                    if t + DL < NT:
                        qkv_tile(t + DL)
                    if t < NT:
                        attn_tile(t)
                        qa_tile(t)
                    if t > 0:
                        outb_tile(t - 1)
                        outa_tile(t - 1)
                        store_tile(t - 1)
        elif p2 == 'c':
            DL = 2
            for t in range(NT + 1):
                with scope(f"p2_{t // 4}"):
                    if t > 0:
                        outb_tile(t - 1)
                        outa_tile(t - 1)
                        store_tile(t - 1)
                    if t < NT:
                        qa_tile(t)
                        attn_tile(t)
                    if t + DL < NT:
                        qkv_tile(t + DL)
        with scope("waitout"):
            for c in ocopies:
                c.wait()

    scratch = [
        pltpu.VMEM((NT, D, 128), BF),
        pltpu.VMEM((NT, D, 128), BF),
        pltpu.VMEM((D, 3 * D), BF),
        pltpu.VMEM((D, 3 * D), BF),
        pltpu.VMEM((D, D), BF),
        pltpu.VMEM((D, D), BF),
        pltpu.VMEM((CT, 2 * D, 128), BF),
        pltpu.VMEM((CT, 3 * D, 128), BF),
        pltpu.VMEM((CT, D, 128), BF),
        pltpu.VMEM((CT, D, 128), BF),
        pltpu.VMEM((CT, D, 128), BF),
        pltpu.VMEM((CT, 3 * D, 128), BF),
        pltpu.VMEM((CT, D, 128), BF),
        pltpu.VMEM((D, D), BF),
        pltpu.VMEM((CT, D, 128), BF),
        pltpu.VMEM((D, 128), F32),
        pltpu.VMEM((NT, D, 128), BF),
        pltpu.VMEM((NT + 1, D, 128), F32 if kf32 else BF),
        pltpu.VMEM((NT + 1, D, 128), F32 if kf32 else BF),
        pltpu.VMEM((NT + 2, 128, 2 * D), BF),
        pltpu.SemaphoreType.DMA((2 * NT,)),
        pltpu.SemaphoreType.DMA((15,)),
        pltpu.SemaphoreType.DMA((NT,)),
    ]

    def f(A_x, A_wqkv, A_wo, B_x, B_wqkv, B_wo):
        out = pl.pallas_call(
            kernel,
            out_shape=jax.ShapeDtypeStruct((S, 2 * D), BF),
            grid=(1,),
            in_specs=[pl.BlockSpec(memory_space=pl.ANY)] * 6,
            out_specs=pl.BlockSpec(memory_space=pl.ANY),
            scratch_shapes=scratch,
            compiler_params=pltpu.CompilerParams(vmem_limit_bytes=110 * 2**20, flags=flags),
        )(A_x[0].T, A_wqkv, A_wo, B_x[0].T, B_wqkv, B_wo)
        return out[None]
    f.__name__ = 'kern'
    return jax.jit(f)


_impl = build(p2='a', kf32=True, split=True, DC=2, DLA=1)


@jax.jit
def pallas_concat_heads__linear_attn_block__sliding_local_dilated__prompt_kernel(
    A_x: jax.Array,
    A_wqkv: jax.Array,
    A_wo: jax.Array,
    B_x: jax.Array,
    B_wqkv: jax.Array,
    B_wo: jax.Array,
):
    return _impl(A_x, A_wqkv, A_wo, B_x, B_wqkv, B_wo)
```

```python
import functools

import jax
import jax.numpy as jnp
import numpy as np
import jax.experimental.pallas as pl
import jax.experimental.pallas.tpu as pltpu

S = 2048
D = 576
DH = 18
W = 8
DIL = 2
NT = S // 128
CT = 5
NG = 4
GR = 144
DC = 2
BF = jnp.bfloat16
F32 = jnp.float32
U32 = jnp.uint32


def _cw(ct):
    return min(128, D - ct * 128)


def _kernel(xa_hbm, wa_hbm, woa_hbm, xb_hbm, wb_hbm, wob_hbm, out_hbm,
            xa_v, xb_v, wa_v, wb_v, woa_v, wob_v, tba, tbb, tbo,
            wqa, wka, wbT, wobT, m_v, mT, zb, pkb, kB, vB, obuf,
            sem_x, sem_w, sem_o):
    def xcopy(src, dst, t, si):
        return pltpu.make_async_copy(
            src.at[:, pl.ds(pl.multiple_of(t * 128, 128), 128)], dst.at[t], sem_x.at[si])

    def colcopy(src, dst, c, si):
        c0 = pl.multiple_of(c * 128, 128)
        return pltpu.make_async_copy(
            src.at[:, pl.ds(c0, 128)], dst.at[:, pl.ds(c0, 128)], sem_w.at[si])

    def rowcopy(src, dst, i, c0, nc, si):
        r0 = pl.multiple_of(i * (D // 2), D // 2)
        return pltpu.make_async_copy(
            src.at[pl.ds(r0, D // 2), pl.ds(c0, nc)],
            dst.at[pl.ds(r0, D // 2), pl.ds(c0, nc)], sem_w.at[si])

    d_wk = (5, lambda i: colcopy(wa_hbm, wa_v, 4 + i, i))
    d_xa0 = (12, lambda i: xcopy(xa_hbm, xa_v, i, i))
    d_xa1 = (4, lambda i: xcopy(xa_hbm, xa_v, 12 + i, 12 + i))
    d_wb = (2, lambda i: rowcopy(wb_hbm, wb_v, i, 0, 3 * D, 5 + i))
    d_wq = (2, lambda i: rowcopy(wa_hbm, wa_v, i, 0, 512, 7 + i))
    d_xb0 = (2, lambda i: xcopy(xb_hbm, xb_v, i, NT + i))
    d_wv = (2, lambda i: rowcopy(wa_hbm, wa_v, i, 2 * D, D, 9 + i))
    d_woa = (2, lambda i: rowcopy(woa_hbm, woa_v, i, 0, D, 11 + i))
    d_wob = (2, lambda i: rowcopy(wob_hbm, wob_v, i, 0, D, 13 + i))
    d_xb1 = (NT - 2, lambda i: xcopy(xb_hbm, xb_v, 2 + i, NT + 2 + i))

    def issue(dsc):
        n, mk = dsc

        def body(i, c):
            mk(i).start()
            return c
        jax.lax.fori_loop(0, n, body, 0)

    def every(dsc):
        return [dsc[1](i) for i in range(dsc[0])]

    def wait(cs):
        for c in cs:
            c.wait()

    cwk = every(d_wk)
    cxa = every(d_xa0) + every(d_xa1)
    cxb = every(d_xb0) + every(d_xb1)
    c_wb, c_wq, c_wv, c_woa, c_wob = (every(x) for x in (d_wb, d_wq, d_wv, d_woa, d_wob))

    zero = pl.program_id(0)
    sub = jax.lax.broadcasted_iota(jnp.int32, (8, 128), 0)
    lane = jax.lax.broadcasted_iota(jnp.int32, (1, 128), 1)
    st = {}

    def transpose_tiles(w_v, tb, n_lo, n_hi):
        for n0 in range(n_lo, n_hi, 128):
            n1 = min(n0 + 128, n_hi)
            for ct in range(CT):
                cw = _cw(ct)
                tb.bitcast(U32)[ct, n0 // 2:n1 // 2, 0:cw] = pltpu.bitcast(
                    w_v[ct * 128:ct * 128 + cw, n0:n1].T, U32)

    def perm_rows(load, row0, pairs=(0, 2)):
        out = [None] * (NG * (DH // 2))
        for g in pairs:
            for d2 in range(DH // 2):
                base = row0 // 2 + g * (GR // 2) + d2
                ev = load(base)
                od = load(base + DH // 2)
                p = (ev & np.uint32(0xFFFF)) | (od << 16)
                q = (ev >> 16) | (od & np.uint32(0xFFFF0000))
                out[g * (DH // 2) + d2] = jnp.where(sub < 4, p, pltpu.roll(q, 4, axis=0))
                out[(g + 1) * (DH // 2) + d2] = jnp.where(sub < 4, pltpu.roll(p, 4, axis=0), q)
        return jnp.concatenate([o for o in out if o is not None], axis=0)

    def gather_perm(dst, dst_row0, tb, src_row0, pairs=(0, 2)):
        tu = tb.bitcast(U32)
        for ct in range(CT):
            for g in pairs:
                w0 = (dst_row0 + g * GR) // 2
                dst.bitcast(U32)[ct, w0:w0 + GR, :] = perm_rows(
                    lambda r: tu[ct, pl.ds(r, 8, stride=DH), :], src_row0, (g,))

    def prep_wob():
        for ct in range(CT):
            cw = _cw(ct)
            tbo.bitcast(U32)[ct, :, 0:cw] = wob_v.bitcast(U32)[:, ct * 128:ct * 128 + cw]
        tu = tbo.bitcast(U32)
        for ct in range(CT):
            cw = _cw(ct)
            full = pltpu.bitcast(
                perm_rows(lambda r: tu[ct, pl.ds(r, 8, stride=DH), :], 0), BF)
            for rt in range(CT):
                rw = _cw(rt)
                wobT.bitcast(U32)[rt, ct * 64:ct * 64 + cw // 2, 0:rw] = pltpu.bitcast(
                    full[rt * 128:rt * 128 + rw, 0:cw].T, U32)

    def lhs(ref, rows=D):
        u = ref.bitcast(U32)
        return jnp.concatenate(
            [pltpu.bitcast(u[c, 0:rows // 2, :], BF) for c in range(CT)], axis=1)[:, :D]

    def xt(ref, t):
        return pltpu.bitcast(ref.bitcast(U32)[t], BF)

    def phi(t):
        return jnp.where(t > 0, t + 1.0, jnp.exp(t)) + 1e-6

    def k_mm(t):
        st[('kt', t)] = jnp.dot(lhs(wka), xt(xa_v, t), preferred_element_type=F32)

    def k_post(t):
        pk = phi(st.pop(('kt', t)))
        st['z'] = pk if 'z' not in st else st['z'] + pk
        pkb[t] = pk.astype(BF)

    def g_block(b):
        tiles = range(4 * b, 4 * b + 4)
        pk = jnp.concatenate([xt(pkb, t) for t in tiles], axis=1)
        xblk = jnp.concatenate([xt(xa_v, t) for t in tiles], axis=1)
        gt = jax.lax.dot_general(pk, xblk, (((1,), (1,)), ((), ())),
                                 preferred_element_type=F32)
        st['g'] = gt if 'g' not in st else st['g'] + gt

    def small_kv():
        z = jnp.sum(st['z'], axis=1, keepdims=True)
        zb[...] = jnp.broadcast_to(z, (D, 128))
        gb = st['g'].astype(BF)
        for g in range(NG):
            n0 = 128 * g
            n1 = min(n0 + 256, D)
            kv = jnp.dot(gb[g * GR:(g + 1) * GR, :], wa_v[:, 2 * D + n0:2 * D + n1],
                         preferred_element_type=F32)
            row = jax.lax.broadcasted_iota(jnp.int32, kv.shape, 0)
            col = jax.lax.broadcasted_iota(jnp.int32, kv.shape, 1) + n0
            same = ((col * 3641) >> 16) == (row & 7) + 8 * g
            st[('kv', g)] = jnp.where(same, kv, 0.0).astype(BF)

    def small_m():
        for g in range(NG):
            n0 = 128 * g
            n1 = min(n0 + 256, D)
            m_v[g * GR:(g + 1) * GR, :] = jnp.dot(
                st.pop(('kv', g)), woa_v[n0:n1, :], preferred_element_type=F32).astype(BF)

    def small_t():
        for rt in range(CT):
            rw = _cw(rt)
            for ct in range(CT):
                cw = _cw(ct)
                mT.bitcast(U32)[rt, ct * 64:ct * 64 + cw // 2, 0:rw] = pltpu.bitcast(
                    m_v[rt * 128:rt * 128 + rw, ct * 128:ct * 128 + cw].T, U32)

    def qkv_tile(t):
        qkv = jnp.dot(lhs(wbT, 3 * D), xt(xb_v, t), preferred_element_type=F32)
        st[('q', t)] = qkv[0:D]
        kB[t] = qkv[D:2 * D]
        vB[t] = qkv[2 * D:3 * D]

    def shifted(prev, cur, w):
        if w == 0:
            return cur
        return pltpu.roll(jnp.where(lane >= 128 - DIL * w, prev, cur), DIL * w, axis=1)

    def attn_tile(t):
        o_parts = []
        q = st.pop(('q', t))
        for g in range(NG):
            logits = [None] * W
            for c in range(DH // DC):
                r0 = g * GR + c * DC * 8
                r1 = r0 + DC * 8
                q3 = q[r0:r1].reshape(DC, 8, 128)
                kc = kB[t, r0:r1, :]
                kp = kB[t - 1, r0:r1, :] if t > 0 else jnp.zeros_like(kc)
                for w in range(W):
                    ks = shifted(kp, kc, w).reshape(DC, 8, 128)
                    part = jnp.sum(q3 * ks, axis=0)
                    logits[w] = part if c == 0 else logits[w] + part
            for w in range(W):
                lw = logits[w] * (DH ** -0.5)
                if t == 0 and w > 0:
                    lw = jnp.where(lane >= DIL * w, lw, -1e9)
                logits[w] = lw
            m = functools.reduce(jnp.maximum, logits)
            es = [jnp.exp(l - m) for l in logits]
            rs = 1.0 / functools.reduce(jnp.add, es)
            ps = [(e * rs)[None] for e in es]
            for c in range(DH // DC):
                r0 = g * GR + c * DC * 8
                r1 = r0 + DC * 8
                vc = vB[t, r0:r1, :]
                vp = vB[t - 1, r0:r1, :] if t > 0 else jnp.zeros_like(vc)
                o = None
                for w in range(W):
                    cw = shifted(vp, vc, w).reshape(DC, 8, 128) * ps[w]
                    o = cw if o is None else o + cw
                o_parts.append(o.reshape(DC * 8, 128))
        ov = jnp.concatenate(o_parts, axis=0).astype(BF)
        for b in range(CT):
            obuf[NT + (t % 2) + zero, 0:_cw(b), 128 * b:128 * (b + 1)] = (
                ov[128 * b:128 * b + _cw(b), :])

    def qa_tile(t):
        pj = phi(jnp.dot(lhs(wqa), xt(xa_v, t), preferred_element_type=F32))
        tt = (pj * zb[...]).reshape(NG, DH, 8, 128)
        den = jnp.sum(tt, axis=1, keepdims=True) + 1e-6
        pn = pj.reshape(NG, DH, 8, 128) * (1.0 / den)
        st[('pqn', t)] = pn.reshape(D, 128).astype(BF)

    def outb_tile(t):
        ov = jnp.concatenate(
            [obuf[NT + (t % 2) + zero, 0:_cw(b), 128 * b:128 * (b + 1)] for b in range(CT)],
            axis=0)
        st[('outb', t)] = jnp.dot(lhs(wobT), ov, preferred_element_type=F32)

    def outa_tile(t):
        st[('outa', t)] = jnp.dot(lhs(mT), st.pop(('pqn', t)), preferred_element_type=F32)

    ocopies = []

    def store_tile(t):
        full = jnp.concatenate([st.pop(('outa', t)), st.pop(('outb', t))], axis=0).astype(BF)
        obuf[t] = full.T
        c = pltpu.make_async_copy(
            obuf.at[t], out_hbm.at[pl.ds(t * 128, 128), :], sem_o.at[t])
        c.start()
        ocopies.append(c)

    for dsc in (d_wk, d_xa0, d_xa1, d_wb, d_wq, d_xb0, d_wv, d_woa, d_wob, d_xb1):
        issue(dsc)

    for i in range(3):
        wait([cwk[i]])
        transpose_tiles(wa_v, tba, 512 + 128 * i, 640 + 128 * i)
    gather_perm(wka, 0, tba, D, (0,))
    for i in range(3, 5):
        wait([cwk[i]])
        transpose_tiles(wa_v, tba, 512 + 128 * i, 640 + 128 * i)
    gather_perm(wka, 0, tba, D, (2,))

    wait(cxa[0:1])
    k_mm(0)
    wait(cxa[1:4])
    k_mm(1)
    k_post(0)
    k_mm(2)
    k_post(1)
    k_mm(3)
    k_post(2)
    wait(cxa[4:8])
    k_mm(4)
    k_post(3)
    for t in range(5, 8):
        k_mm(t)
        k_post(t - 1)
    g_block(0)
    wait(cxa[8:16])
    k_post(7)
    for t in range(8, 12):
        k_mm(t)
        if t > 8:
            k_post(t - 1)
    wait(c_wb)
    transpose_tiles(wb_v, tbb, 0, 640)
    k_post(11)
    g_block(1)
    gather_perm(wbT, 0, tbb, 0)
    transpose_tiles(wb_v, tbb, 640, 1152)
    for t in range(12, 16):
        k_mm(t)
        k_post(t)
    gather_perm(wbT, D, tbb, D)
    transpose_tiles(wb_v, tbb, 1152, 1728)
    gather_perm(wbT, 2 * D, tbb, 2 * D)
    g_block(2)
    wait(c_wq + cxb[0:2] + c_wv + c_woa + c_wob + cxb[2:16])
    qkv_tile(0)
    transpose_tiles(wa_v, tba, 0, 512)
    gather_perm(wqa, 0, tba, 0)
    g_block(3)
    prep_wob()
    small_kv()
    small_m()
    small_t()

    for t in range(NT):
        if t + 1 < NT:
            qkv_tile(t + 1)
        qa_tile(t)
        attn_tile(t)
        outb_tile(t)
        outa_tile(t)
        store_tile(t)
    wait(ocopies)


def _scratch():
    return [
        pltpu.VMEM((NT, D, 128), BF),
        pltpu.VMEM((NT, D, 128), BF),
        pltpu.VMEM((D, 3 * D), BF),
        pltpu.VMEM((D, 3 * D), BF),
        pltpu.VMEM((D, D), BF),
        pltpu.VMEM((D, D), BF),
        pltpu.VMEM((CT, 2 * D, 128), BF),
        pltpu.VMEM((CT, 3 * D, 128), BF),
        pltpu.VMEM((CT, D, 128), BF),
        pltpu.VMEM((CT, D, 128), BF),
        pltpu.VMEM((CT, D, 128), BF),
        pltpu.VMEM((CT, 3 * D, 128), BF),
        pltpu.VMEM((CT, D, 128), BF),
        pltpu.VMEM((D, D), BF),
        pltpu.VMEM((CT, D, 128), BF),
        pltpu.VMEM((D, 128), F32),
        pltpu.VMEM((NT, D, 128), BF),
        pltpu.VMEM((NT, D, 128), F32),
        pltpu.VMEM((NT, D, 128), F32),
        pltpu.VMEM((NT + 2, 128, 2 * D), BF),
        pltpu.SemaphoreType.DMA((2 * NT,)),
        pltpu.SemaphoreType.DMA((15,)),
        pltpu.SemaphoreType.DMA((NT,)),
    ]


@jax.jit
def pallas_concat_heads__linear_attn_block__sliding_local_dilated__prompt_kernel(
    A_x: jax.Array,
    A_wqkv: jax.Array,
    A_wo: jax.Array,
    B_x: jax.Array,
    B_wqkv: jax.Array,
    B_wo: jax.Array,
):
    out = pl.pallas_call(
        _kernel,
        out_shape=jax.ShapeDtypeStruct((S, 2 * D), BF),
        grid=(1,),
        in_specs=[pl.BlockSpec(memory_space=pl.ANY)] * 6,
        out_specs=pl.BlockSpec(memory_space=pl.ANY),
        scratch_shapes=_scratch(),
        compiler_params=pltpu.CompilerParams(vmem_limit_bytes=110 * 2**20),
    )(A_x[0].T, A_wqkv, A_wo, B_x[0].T, B_wqkv, B_wo)
    return out[None]
```

```python
import functools

import jax
import jax.numpy as jnp
import numpy as np
import jax.experimental.pallas as pl
import jax.experimental.pallas.tpu as pltpu

S = 2048
D = 576
DH = 18
W = 8
DIL = 2
NT = S // 128
CT = 5
NG = 4
GR = 144
DC = 2
BF = jnp.bfloat16
F32 = jnp.float32
U32 = jnp.uint32


def _cw(ct):
    return min(128, D - ct * 128)


def _kernel(xa_hbm, wa_hbm, woa_hbm, xb_hbm, wb_hbm, wob_hbm, out_hbm,
            xa_v, xb_v, wa_v, wb_v, woa_v, wob_v, tba, tbb, tbo,
            wqa, wka, wbT, wobT, m_v, mT, zb, pkb, kB, vB, obuf,
            sems):
    def xcopy(src, dst, t, si):
        return pltpu.make_async_copy(
            src.at[:, pl.ds(pl.multiple_of(t * 128, 128), 128)], dst.at[t], sems.at[si])

    def colcopy(src, dst, c, si):
        c0 = pl.multiple_of(c * 128, 128)
        return pltpu.make_async_copy(
            src.at[:, pl.ds(c0, 128)], dst.at[:, pl.ds(c0, 128)], sems.at[si])

    def rowcopy(src, dst, i, c0, nc, si):
        r0 = pl.multiple_of(i * (D // 2), D // 2)
        return pltpu.make_async_copy(
            src.at[pl.ds(r0, D // 2), pl.ds(c0, nc)],
            dst.at[pl.ds(r0, D // 2), pl.ds(c0, nc)], sems.at[si])

    d_wk = (5, lambda i: colcopy(wa_hbm, wa_v, 4 + i, i))
    d_xa0 = (1, lambda i: xcopy(xa_hbm, xa_v, i, 5))
    d_xa1 = (3, lambda i: xcopy(xa_hbm, xa_v, 1 + i, 6))
    d_xa4 = (4, lambda i: xcopy(xa_hbm, xa_v, 4 + i, 7))
    d_xa8 = (8, lambda i: xcopy(xa_hbm, xa_v, 8 + i, 8))
    d_wb = (2, lambda i: rowcopy(wb_hbm, wb_v, i, 0, 3 * D, 9))
    d_wq = (2, lambda i: rowcopy(wa_hbm, wa_v, i, 0, 512, 10))
    d_xb0 = (2, lambda i: xcopy(xb_hbm, xb_v, i, 10))
    d_wv = (2, lambda i: rowcopy(wa_hbm, wa_v, i, 2 * D, D, 10))
    d_woa = (2, lambda i: rowcopy(woa_hbm, woa_v, i, 0, D, 10))
    d_wob = (2, lambda i: rowcopy(wob_hbm, wob_v, i, 0, D, 10))
    d_xb1 = (NT - 2, lambda i: xcopy(xb_hbm, xb_v, 2 + i, 10))

    def issue(dsc):
        n, mk = dsc

        def body(i, c):
            mk(i).start()
            return c
        jax.lax.fori_loop(0, n, body, 0)

    def every(dsc):
        return [dsc[1](i) for i in range(dsc[0])]

    def wait(cs):
        for c in cs:
            c.wait()

    cwk = every(d_wk)
    cxa = every(d_xa0) + every(d_xa1) + every(d_xa4) + every(d_xa8)
    cxb = every(d_xb0) + every(d_xb1)
    c_wb, c_wq, c_wv, c_woa, c_wob = (every(x) for x in (d_wb, d_wq, d_wv, d_woa, d_wob))

    zero = pl.program_id(0)
    sub = jax.lax.broadcasted_iota(jnp.int32, (8, 128), 0)
    lane = jax.lax.broadcasted_iota(jnp.int32, (1, 128), 1)
    st = {}

    def transpose_tiles(w_v, tb, n_lo, n_hi):
        for n0 in range(n_lo, n_hi, 128):
            n1 = min(n0 + 128, n_hi)
            for ct in range(CT):
                cw = _cw(ct)
                tb.bitcast(U32)[ct, n0 // 2:n1 // 2, 0:cw] = pltpu.bitcast(
                    w_v[ct * 128:ct * 128 + cw, n0:n1].T, U32)

    def perm_rows(load, row0, pairs=(0, 2)):
        out = [None] * (NG * (DH // 2))
        for g in pairs:
            for d2 in range(DH // 2):
                base = row0 // 2 + g * (GR // 2) + d2
                ev = load(base)
                od = load(base + DH // 2)
                p = (ev & np.uint32(0xFFFF)) | (od << 16)
                q = (ev >> 16) | (od & np.uint32(0xFFFF0000))
                out[g * (DH // 2) + d2] = jnp.where(sub < 4, p, pltpu.roll(q, 4, axis=0))
                out[(g + 1) * (DH // 2) + d2] = jnp.where(sub < 4, pltpu.roll(p, 4, axis=0), q)
        return jnp.concatenate([o for o in out if o is not None], axis=0)

    def gather_perm(dst, dst_row0, tb, src_row0, pairs=(0, 2)):
        tu = tb.bitcast(U32)
        for ct in range(CT):
            for g in pairs:
                w0 = (dst_row0 + g * GR) // 2
                dst.bitcast(U32)[ct, w0:w0 + GR, :] = perm_rows(
                    lambda r: tu[ct, pl.ds(r, 8, stride=DH), :], src_row0, (g,))

    def prep_wob():
        for ct in range(CT):
            cw = _cw(ct)
            tbo.bitcast(U32)[ct, :, 0:cw] = wob_v.bitcast(U32)[:, ct * 128:ct * 128 + cw]
        tu = tbo.bitcast(U32)
        for ct in range(CT):
            cw = _cw(ct)
            full = pltpu.bitcast(
                perm_rows(lambda r: tu[ct, pl.ds(r, 8, stride=DH), :], 0), BF)
            for rt in range(CT):
                rw = _cw(rt)
                wobT.bitcast(U32)[rt, ct * 64:ct * 64 + cw // 2, 0:rw] = pltpu.bitcast(
                    full[rt * 128:rt * 128 + rw, 0:cw].T, U32)

    def lhs(ref, rows=D):
        u = ref.bitcast(U32)
        return jnp.concatenate(
            [pltpu.bitcast(u[c, 0:rows // 2, :], BF) for c in range(CT)], axis=1)[:, :D]

    def xt(ref, t):
        return pltpu.bitcast(ref.bitcast(U32)[t], BF)

    def phi(t):
        return jnp.where(t > 0, t + 1.0, jnp.exp(t)) + 1e-6

    def k_mm(t):
        st[('kt', t)] = jnp.dot(lhs(wka), xt(xa_v, t), preferred_element_type=F32)

    def k_post(t):
        pk = phi(st.pop(('kt', t)))
        st['z'] = pk if 'z' not in st else st['z'] + pk
        pkb[t] = pk.astype(BF)

    def g_block(b):
        tiles = range(4 * b, 4 * b + 4)
        pk = jnp.concatenate([xt(pkb, t) for t in tiles], axis=1)
        xblk = jnp.concatenate([xt(xa_v, t) for t in tiles], axis=1)
        gt = jax.lax.dot_general(pk, xblk, (((1,), (1,)), ((), ())),
                                 preferred_element_type=F32)
        st['g'] = gt if 'g' not in st else st['g'] + gt

    def small_kv():
        z = jnp.sum(st['z'], axis=1, keepdims=True)
        zb[...] = jnp.broadcast_to(z, (D, 128))
        gb = st['g'].astype(BF)
        for g in range(NG):
            n0 = 128 * g
            n1 = min(n0 + 256, D)
            kv = jnp.dot(gb[g * GR:(g + 1) * GR, :], wa_v[:, 2 * D + n0:2 * D + n1],
                         preferred_element_type=F32)
            row = jax.lax.broadcasted_iota(jnp.int32, kv.shape, 0)
            col = jax.lax.broadcasted_iota(jnp.int32, kv.shape, 1) + n0
            same = ((col * 3641) >> 16) == (row & 7) + 8 * g
            st[('kv', g)] = jnp.where(same, kv, 0.0).astype(BF)

    def small_m():
        for g in range(NG):
            n0 = 128 * g
            n1 = min(n0 + 256, D)
            m_v[g * GR:(g + 1) * GR, :] = jnp.dot(
                st.pop(('kv', g)), woa_v[n0:n1, :], preferred_element_type=F32).astype(BF)

    def small_t():
        for rt in range(CT):
            rw = _cw(rt)
            for ct in range(CT):
                cw = _cw(ct)
                mT.bitcast(U32)[rt, ct * 64:ct * 64 + cw // 2, 0:rw] = pltpu.bitcast(
                    m_v[rt * 128:rt * 128 + rw, ct * 128:ct * 128 + cw].T, U32)

    def qkv_tile(t):
        qkv = jnp.dot(lhs(wbT, 3 * D), xt(xb_v, t), preferred_element_type=F32)
        st[('q', t)] = qkv[0:D]
        kB[t] = qkv[D:2 * D]
        vB[t] = qkv[2 * D:3 * D]

    def shifted(prev, cur, w):
        if w == 0:
            return cur
        return pltpu.roll(jnp.where(lane >= 128 - DIL * w, prev, cur), DIL * w, axis=1)

    def attn_tile(t):
        o_parts = []
        q = st.pop(('q', t))
        for g in range(NG):
            logits = [None] * W
            for c in range(DH // DC):
                r0 = g * GR + c * DC * 8
                r1 = r0 + DC * 8
                q3 = q[r0:r1].reshape(DC, 8, 128)
                kc = kB[t, r0:r1, :]
                kp = kB[t - 1, r0:r1, :] if t > 0 else jnp.zeros_like(kc)
                for w in range(W):
                    ks = shifted(kp, kc, w).reshape(DC, 8, 128)
                    part = jnp.sum(q3 * ks, axis=0)
                    logits[w] = part if c == 0 else logits[w] + part
            for w in range(W):
                lw = logits[w] * (DH ** -0.5)
                if t == 0 and w > 0:
                    lw = jnp.where(lane >= DIL * w, lw, -1e9)
                logits[w] = lw
            m = functools.reduce(jnp.maximum, logits)
            es = [jnp.exp(l - m) for l in logits]
            rs = 1.0 / functools.reduce(jnp.add, es)
            ps = [(e * rs)[None] for e in es]
            for c in range(DH // DC):
                r0 = g * GR + c * DC * 8
                r1 = r0 + DC * 8
                vc = vB[t, r0:r1, :]
                vp = vB[t - 1, r0:r1, :] if t > 0 else jnp.zeros_like(vc)
                o = None
                for w in range(W):
                    cw = shifted(vp, vc, w).reshape(DC, 8, 128) * ps[w]
                    o = cw if o is None else o + cw
                o_parts.append(o.reshape(DC * 8, 128))
        ov = jnp.concatenate(o_parts, axis=0).astype(BF)
        for b in range(CT):
            obuf[NT + (t % 2) + zero, 0:_cw(b), 128 * b:128 * (b + 1)] = (
                ov[128 * b:128 * b + _cw(b), :])

    def qa_tile(t):
        pj = phi(jnp.dot(lhs(wqa), xt(xa_v, t), preferred_element_type=F32))
        tt = (pj * zb[...]).reshape(NG, DH, 8, 128)
        den = jnp.sum(tt, axis=1, keepdims=True) + 1e-6
        pn = pj.reshape(NG, DH, 8, 128) * (1.0 / den)
        st[('pqn', t)] = pn.reshape(D, 128).astype(BF)

    def outb_tile(t):
        ov = jnp.concatenate(
            [obuf[NT + (t % 2) + zero, 0:_cw(b), 128 * b:128 * (b + 1)] for b in range(CT)],
            axis=0)
        st[('outb', t)] = jnp.dot(lhs(wobT), ov, preferred_element_type=F32)

    def outa_tile(t):
        st[('outa', t)] = jnp.dot(lhs(mT), st.pop(('pqn', t)), preferred_element_type=F32)

    ocopies = []

    def store_tile(t):
        full = jnp.concatenate([st.pop(('outa', t)), st.pop(('outb', t))], axis=0).astype(BF)
        cuts = (0, 512, 640, 2 * D) if t == NT - 1 else (0, 2 * D)
        for c0, c1 in reversed(list(zip(cuts[:-1], cuts[1:]))):
            obuf[t, :, c0:c1] = full[c0:c1].T
            c = pltpu.make_async_copy(
                obuf.at[t, :, pl.ds(c0, c1 - c0)],
                out_hbm.at[pl.ds(t * 128, 128), pl.ds(c0, c1 - c0)], sems.at[11])
            c.start()
            ocopies.append(c)

    for dsc in (d_wk, d_xa0, d_xa1, d_xa4, d_xa8, d_wb,
                d_wq, d_xb0, d_wv, d_woa, d_wob, d_xb1):
        issue(dsc)

    for i in range(3):
        wait([cwk[i]])
        transpose_tiles(wa_v, tba, 512 + 128 * i, 640 + 128 * i)
    gather_perm(wka, 0, tba, D, (0,))
    for i in range(3, 5):
        wait([cwk[i]])
        transpose_tiles(wa_v, tba, 512 + 128 * i, 640 + 128 * i)
    gather_perm(wka, 0, tba, D, (2,))

    wait(cxa[0:1])
    k_mm(0)
    wait(cxa[1:4])
    k_mm(1)
    k_post(0)
    k_mm(2)
    k_post(1)
    k_mm(3)
    k_post(2)
    wait(cxa[4:8])
    k_mm(4)
    k_post(3)
    for t in range(5, 8):
        k_mm(t)
        k_post(t - 1)
    g_block(0)
    wait(cxa[8:16])
    k_post(7)
    for t in range(8, 12):
        k_mm(t)
        if t > 8:
            k_post(t - 1)
    wait(c_wb)
    transpose_tiles(wb_v, tbb, 0, 640)
    k_post(11)
    g_block(1)
    gather_perm(wbT, 0, tbb, 0)
    transpose_tiles(wb_v, tbb, 640, 1152)
    for t in range(12, 16):
        k_mm(t)
        k_post(t)
    gather_perm(wbT, D, tbb, D)
    transpose_tiles(wb_v, tbb, 1152, 1728)
    gather_perm(wbT, 2 * D, tbb, 2 * D)
    g_block(2)
    wait(c_wq + cxb[0:2] + c_wv + c_woa + c_wob + cxb[2:16])
    qkv_tile(0)
    transpose_tiles(wa_v, tba, 0, 512)
    gather_perm(wqa, 0, tba, 0)
    g_block(3)
    prep_wob()
    small_kv()
    small_m()
    small_t()

    for t in range(NT):
        if t + 1 < NT:
            qkv_tile(t + 1)
        qa_tile(t)
        attn_tile(t)
        outb_tile(t)
        outa_tile(t)
        store_tile(t)
    wait(ocopies)


def _scratch():
    return [
        pltpu.VMEM((NT, D, 128), BF),
        pltpu.VMEM((NT, D, 128), BF),
        pltpu.VMEM((D, 3 * D), BF),
        pltpu.VMEM((D, 3 * D), BF),
        pltpu.VMEM((D, D), BF),
        pltpu.VMEM((D, D), BF),
        pltpu.VMEM((CT, 2 * D, 128), BF),
        pltpu.VMEM((CT, 3 * D, 128), BF),
        pltpu.VMEM((CT, D, 128), BF),
        pltpu.VMEM((CT, D, 128), BF),
        pltpu.VMEM((CT, D, 128), BF),
        pltpu.VMEM((CT, 3 * D, 128), BF),
        pltpu.VMEM((CT, D, 128), BF),
        pltpu.VMEM((D, D), BF),
        pltpu.VMEM((CT, D, 128), BF),
        pltpu.VMEM((D, 128), F32),
        pltpu.VMEM((NT, D, 128), BF),
        pltpu.VMEM((NT, D, 128), F32),
        pltpu.VMEM((NT, D, 128), F32),
        pltpu.VMEM((NT + 2, 128, 2 * D), BF),
        pltpu.SemaphoreType.DMA((12,)),
    ]


@jax.jit
def pallas_concat_heads__linear_attn_block__sliding_local_dilated__prompt_kernel(
    A_x: jax.Array,
    A_wqkv: jax.Array,
    A_wo: jax.Array,
    B_x: jax.Array,
    B_wqkv: jax.Array,
    B_wo: jax.Array,
):
    out = pl.pallas_call(
        _kernel,
        out_shape=jax.ShapeDtypeStruct((S, 2 * D), BF),
        grid=(1,),
        in_specs=[pl.BlockSpec(memory_space=pl.ANY)] * 6,
        out_specs=pl.BlockSpec(memory_space=pl.ANY),
        scratch_shapes=_scratch(),
        compiler_params=pltpu.CompilerParams(vmem_limit_bytes=110 * 2**20),
    )(A_x[0].T, A_wqkv, A_wo, B_x[0].T, B_wqkv, B_wo)
    return out[None]
```

```python
import functools

import jax
import jax.numpy as jnp
import numpy as np
import jax.experimental.pallas as pl
import jax.experimental.pallas.tpu as pltpu

S = 2048
D = 576
DH = 18
W = 8
DIL = 2
NT = S // 128
CT = 5
NG = 4
GR = 144
DC = 2
BF = jnp.bfloat16
F32 = jnp.float32
U32 = jnp.uint32


def _cw(ct):
    return min(128, D - ct * 128)


def _kernel(xa_hbm, wa_hbm, woa_hbm, xb_hbm, wb_hbm, wob_hbm, out_hbm,
            xa_v, xb_v, wa_v, wb_v, woa_v, wob_v, tba, tbb, tbo,
            wqa, wka, wbT, wobT, m_v, mT, zb, pkb, kB, vB, obuf,
            sems):
    def xcopy(src, dst, t, si):
        return pltpu.make_async_copy(
            src.at[:, pl.ds(pl.multiple_of(t * 128, 128), 128)], dst.at[t], sems.at[si])

    def colcopy(src, dst, c, si):
        c0 = pl.multiple_of(c * 128, 128)
        return pltpu.make_async_copy(
            src.at[:, pl.ds(c0, 128)], dst.at[:, pl.ds(c0, 128)], sems.at[si])

    def rowcopy(src, dst, i, c0, nc, si):
        r0 = pl.multiple_of(i * (D // 2), D // 2)
        return pltpu.make_async_copy(
            src.at[pl.ds(r0, D // 2), pl.ds(c0, nc)],
            dst.at[pl.ds(r0, D // 2), pl.ds(c0, nc)], sems.at[si])

    d_wk = (5, lambda i: colcopy(wa_hbm, wa_v, 4 + i, i))
    d_xa0 = (1, lambda i: xcopy(xa_hbm, xa_v, i, 5))
    d_xa1 = (3, lambda i: xcopy(xa_hbm, xa_v, 1 + i, 6))
    d_xa4 = (4, lambda i: xcopy(xa_hbm, xa_v, 4 + i, 7))
    d_xa8 = (8, lambda i: xcopy(xa_hbm, xa_v, 8 + i, 8))
    d_wb = (2, lambda i: rowcopy(wb_hbm, wb_v, i, 0, 3 * D, 9))
    d_wq = (2, lambda i: rowcopy(wa_hbm, wa_v, i, 0, 512, 10))
    d_xb0 = (2, lambda i: xcopy(xb_hbm, xb_v, i, 10))
    d_wv = (2, lambda i: rowcopy(wa_hbm, wa_v, i, 2 * D, D, 10))
    d_woa = (2, lambda i: rowcopy(woa_hbm, woa_v, i, 0, D, 10))
    d_wob = (2, lambda i: rowcopy(wob_hbm, wob_v, i, 0, D, 10))
    d_xb1 = (NT - 2, lambda i: xcopy(xb_hbm, xb_v, 2 + i, 10))

    def issue(dsc):
        n, mk = dsc

        def body(i, c):
            mk(i).start()
            return c
        jax.lax.fori_loop(0, n, body, 0)

    def every(dsc):
        return [dsc[1](i) for i in range(dsc[0])]

    def wait(cs):
        for c in cs:
            c.wait()

    cwk = every(d_wk)
    cxa = every(d_xa0) + every(d_xa1) + every(d_xa4) + every(d_xa8)
    cxb = every(d_xb0) + every(d_xb1)
    c_wb, c_wq, c_wv, c_woa, c_wob = (every(x) for x in (d_wb, d_wq, d_wv, d_woa, d_wob))

    zero = pl.program_id(0)
    sub = jax.lax.broadcasted_iota(jnp.int32, (8, 128), 0)
    lane = jax.lax.broadcasted_iota(jnp.int32, (1, 128), 1)
    st = {}

    def transpose_tiles(w_v, tb, n_lo, n_hi):
        for n0 in range(n_lo, n_hi, 128):
            n1 = min(n0 + 128, n_hi)
            for ct in range(CT):
                cw = _cw(ct)
                tb.bitcast(U32)[ct, n0 // 2:n1 // 2, 0:cw] = pltpu.bitcast(
                    w_v[ct * 128:ct * 128 + cw, n0:n1].T, U32)

    def perm_rows(load, row0, pairs=(0, 2)):
        out = [None] * (NG * (DH // 2))
        for g in pairs:
            for d2 in range(DH // 2):
                base = row0 // 2 + g * (GR // 2) + d2
                ev = load(base)
                od = load(base + DH // 2)
                p = (ev & np.uint32(0xFFFF)) | (od << 16)
                q = (ev >> 16) | (od & np.uint32(0xFFFF0000))
                out[g * (DH // 2) + d2] = jnp.where(sub < 4, p, pltpu.roll(q, 4, axis=0))
                out[(g + 1) * (DH // 2) + d2] = jnp.where(sub < 4, pltpu.roll(p, 4, axis=0), q)
        return jnp.concatenate([o for o in out if o is not None], axis=0)

    def gather_perm(dst, dst_row0, tb, src_row0, pairs=(0, 2)):
        tu = tb.bitcast(U32)
        for ct in range(CT):
            for g in pairs:
                w0 = (dst_row0 + g * GR) // 2
                dst.bitcast(U32)[ct, w0:w0 + GR, :] = perm_rows(
                    lambda r: tu[ct, pl.ds(r, 8, stride=DH), :], src_row0, (g,))

    def prep_wob():
        for ct in range(CT):
            cw = _cw(ct)
            tbo.bitcast(U32)[ct, :, 0:cw] = wob_v.bitcast(U32)[:, ct * 128:ct * 128 + cw]
        tu = tbo.bitcast(U32)
        for ct in range(CT):
            cw = _cw(ct)
            full = pltpu.bitcast(
                perm_rows(lambda r: tu[ct, pl.ds(r, 8, stride=DH), :], 0), BF)
            for rt in range(CT):
                rw = _cw(rt)
                wobT.bitcast(U32)[rt, ct * 64:ct * 64 + cw // 2, 0:rw] = pltpu.bitcast(
                    full[rt * 128:rt * 128 + rw, 0:cw].T, U32)

    def lhs(ref, rows=D):
        u = ref.bitcast(U32)
        return jnp.concatenate(
            [pltpu.bitcast(u[c, 0:rows // 2, :], BF) for c in range(CT)], axis=1)[:, :D]

    def xt(ref, t):
        return pltpu.bitcast(ref.bitcast(U32)[t], BF)

    def phi(t):
        return jnp.where(t > 0, t + 1.0, jnp.exp(t)) + 1e-6

    def k_mm(t):
        st[('kt', t)] = jnp.dot(lhs(wka), xt(xa_v, t), preferred_element_type=F32)

    def k_post(t):
        pk = phi(st.pop(('kt', t)))
        st['z'] = pk if 'z' not in st else st['z'] + pk
        pkb[t] = pk.astype(BF)

    def g_block(b):
        tiles = range(4 * b, 4 * b + 4)
        pk = jnp.concatenate([xt(pkb, t) for t in tiles], axis=1)
        xblk = jnp.concatenate([xt(xa_v, t) for t in tiles], axis=1)
        gt = jax.lax.dot_general(pk, xblk, (((1,), (1,)), ((), ())),
                                 preferred_element_type=F32)
        st['g'] = gt if 'g' not in st else st['g'] + gt

    def small_kv():
        z = jnp.sum(st['z'], axis=1, keepdims=True)
        zb[...] = jnp.broadcast_to(z, (D, 128))
        gb = st['g'].astype(BF)
        for g in range(NG):
            n0 = 128 * g
            n1 = min(n0 + 256, D)
            kv = jnp.dot(gb[g * GR:(g + 1) * GR, :], wa_v[:, 2 * D + n0:2 * D + n1],
                         preferred_element_type=F32)
            row = jax.lax.broadcasted_iota(jnp.int32, kv.shape, 0)
            col = jax.lax.broadcasted_iota(jnp.int32, kv.shape, 1) + n0
            same = ((col * 3641) >> 16) == (row & 7) + 8 * g
            st[('kv', g)] = jnp.where(same, kv, 0.0).astype(BF)

    def small_m():
        for g in range(NG):
            n0 = 128 * g
            n1 = min(n0 + 256, D)
            m_v[g * GR:(g + 1) * GR, :] = jnp.dot(
                st.pop(('kv', g)), woa_v[n0:n1, :], preferred_element_type=F32).astype(BF)

    def small_t():
        for rt in range(CT):
            rw = _cw(rt)
            for ct in range(CT):
                cw = _cw(ct)
                mT.bitcast(U32)[rt, ct * 64:ct * 64 + cw // 2, 0:rw] = pltpu.bitcast(
                    m_v[rt * 128:rt * 128 + rw, ct * 128:ct * 128 + cw].T, U32)

    def qkv_tile(t):
        qkv = jnp.dot(lhs(wbT, 3 * D), xt(xb_v, t), preferred_element_type=F32)
        st[('q', t)] = qkv[0:D]
        kB[t] = qkv[D:2 * D]
        vB[t] = qkv[2 * D:3 * D]

    def shifted(prev, cur, w):
        if w == 0:
            return cur
        return pltpu.roll(jnp.where(lane >= 128 - DIL * w, prev, cur), DIL * w, axis=1)

    def attn_tile(t):
        o_parts = []
        q = st.pop(('q', t))
        for g in range(NG):
            logits = [None] * W
            for c in range(DH // DC):
                r0 = g * GR + c * DC * 8
                r1 = r0 + DC * 8
                q3 = q[r0:r1].reshape(DC, 8, 128)
                kc = kB[t, r0:r1, :]
                kp = kB[t - 1, r0:r1, :] if t > 0 else jnp.zeros_like(kc)
                for w in range(W):
                    ks = shifted(kp, kc, w).reshape(DC, 8, 128)
                    part = jnp.sum(q3 * ks, axis=0)
                    logits[w] = part if c == 0 else logits[w] + part
            for w in range(W):
                lw = logits[w] * (DH ** -0.5)
                if t == 0 and w > 0:
                    lw = jnp.where(lane >= DIL * w, lw, -1e9)
                logits[w] = lw
            m = functools.reduce(jnp.maximum, logits)
            es = [jnp.exp(l - m) for l in logits]
            rs = 1.0 / functools.reduce(jnp.add, es)
            ps = [(e * rs)[None] for e in es]
            for c in range(DH // DC):
                r0 = g * GR + c * DC * 8
                r1 = r0 + DC * 8
                vc = vB[t, r0:r1, :]
                vp = vB[t - 1, r0:r1, :] if t > 0 else jnp.zeros_like(vc)
                o = None
                for w in range(W):
                    cw = shifted(vp, vc, w).reshape(DC, 8, 128) * ps[w]
                    o = cw if o is None else o + cw
                o_parts.append(o.reshape(DC * 8, 128))
        ov = jnp.concatenate(o_parts, axis=0).astype(BF)
        for b in range(CT):
            obuf[NT + (t % 2) + zero, 0:_cw(b), 128 * b:128 * (b + 1)] = (
                ov[128 * b:128 * b + _cw(b), :])

    def qa_tile(t):
        pj = phi(jnp.dot(lhs(wqa), xt(xa_v, t), preferred_element_type=F32))
        tt = (pj * zb[...]).reshape(NG, DH, 8, 128)
        den = jnp.sum(tt, axis=1, keepdims=True) + 1e-6
        pn = pj.reshape(NG, DH, 8, 128) * (1.0 / den)
        st[('pqn', t)] = pn.reshape(D, 128).astype(BF)

    def outb_tile(t):
        ov = jnp.concatenate(
            [obuf[NT + (t % 2) + zero, 0:_cw(b), 128 * b:128 * (b + 1)] for b in range(CT)],
            axis=0)
        st[('outb', t)] = jnp.dot(lhs(wobT), ov, preferred_element_type=F32)

    def outa_tile(t):
        st[('outa', t)] = jnp.dot(lhs(mT), st.pop(('pqn', t)), preferred_element_type=F32)

    ocopies = []

    def store_tile(t):
        full = jnp.concatenate([st.pop(('outa', t)), st.pop(('outb', t))], axis=0).astype(BF)
        cuts = (0, 512, 640, 2 * D) if t == NT - 1 else (0, 2 * D)
        for c0, c1 in reversed(list(zip(cuts[:-1], cuts[1:]))):
            obuf[t, :, c0:c1] = full[c0:c1].T
            c = pltpu.make_async_copy(
                obuf.at[t, :, pl.ds(c0, c1 - c0)],
                out_hbm.at[pl.ds(t * 128, 128), pl.ds(c0, c1 - c0)], sems.at[11])
            c.start()
            ocopies.append(c)

    for dsc in (d_wk, d_xa0, d_xa1, d_xa4, d_xa8, d_wb,
                d_wq, d_xb0, d_wv, d_woa, d_wob, d_xb1):
        issue(dsc)

    for i in range(3):
        wait([cwk[i]])
        transpose_tiles(wa_v, tba, 512 + 128 * i, 640 + 128 * i)
    gather_perm(wka, 0, tba, D, (0,))
    for i in range(3, 5):
        wait([cwk[i]])
        transpose_tiles(wa_v, tba, 512 + 128 * i, 640 + 128 * i)
    gather_perm(wka, 0, tba, D, (2,))

    wait(cxa[0:1])
    k_mm(0)
    wait(cxa[1:4])
    k_mm(1)
    k_post(0)
    k_mm(2)
    k_post(1)
    k_mm(3)
    k_post(2)
    wait(cxa[4:8])
    k_mm(4)
    k_post(3)
    for t in range(5, 8):
        k_mm(t)
        k_post(t - 1)
    k_post(7)
    g_block(0)
    g_block(1)
    wait(cxa[8:16] + c_wb)
    transpose_tiles(wb_v, tbb, 0, 640)
    for t in range(8, 12):
        k_mm(t)
        k_post(t)
    gather_perm(wbT, 0, tbb, 0)
    transpose_tiles(wb_v, tbb, 640, 1152)
    for t in range(12, 16):
        k_mm(t)
        k_post(t)
    gather_perm(wbT, D, tbb, D)
    transpose_tiles(wb_v, tbb, 1152, 1728)
    gather_perm(wbT, 2 * D, tbb, 2 * D)
    g_block(2)
    wait(c_wq + cxb[0:2] + c_wv + c_woa + c_wob + cxb[2:16])
    qkv_tile(0)
    transpose_tiles(wa_v, tba, 0, 512)
    gather_perm(wqa, 0, tba, 0)
    g_block(3)
    prep_wob()
    small_kv()
    small_m()
    small_t()

    for t in range(NT):
        if t + 1 < NT:
            qkv_tile(t + 1)
        qa_tile(t)
        attn_tile(t)
        outb_tile(t)
        outa_tile(t)
        store_tile(t)
    wait(ocopies)


def _scratch():
    return [
        pltpu.VMEM((NT, D, 128), BF),
        pltpu.VMEM((NT, D, 128), BF),
        pltpu.VMEM((D, 3 * D), BF),
        pltpu.VMEM((D, 3 * D), BF),
        pltpu.VMEM((D, D), BF),
        pltpu.VMEM((D, D), BF),
        pltpu.VMEM((CT, 2 * D, 128), BF),
        pltpu.VMEM((CT, 3 * D, 128), BF),
        pltpu.VMEM((CT, D, 128), BF),
        pltpu.VMEM((CT, D, 128), BF),
        pltpu.VMEM((CT, D, 128), BF),
        pltpu.VMEM((CT, 3 * D, 128), BF),
        pltpu.VMEM((CT, D, 128), BF),
        pltpu.VMEM((D, D), BF),
        pltpu.VMEM((CT, D, 128), BF),
        pltpu.VMEM((D, 128), F32),
        pltpu.VMEM((NT, D, 128), BF),
        pltpu.VMEM((NT, D, 128), F32),
        pltpu.VMEM((NT, D, 128), F32),
        pltpu.VMEM((NT + 2, 128, 2 * D), BF),
        pltpu.SemaphoreType.DMA((12,)),
    ]


@jax.jit
def pallas_concat_heads__linear_attn_block__sliding_local_dilated__prompt_kernel(
    A_x: jax.Array,
    A_wqkv: jax.Array,
    A_wo: jax.Array,
    B_x: jax.Array,
    B_wqkv: jax.Array,
    B_wo: jax.Array,
):
    out = pl.pallas_call(
        _kernel,
        out_shape=jax.ShapeDtypeStruct((S, 2 * D), BF),
        grid=(1,),
        in_specs=[pl.BlockSpec(memory_space=pl.ANY)] * 6,
        out_specs=pl.BlockSpec(memory_space=pl.ANY),
        scratch_shapes=_scratch(),
        compiler_params=pltpu.CompilerParams(vmem_limit_bytes=110 * 2**20),
    )(A_x[0].T, A_wqkv, A_wo, B_x[0].T, B_wqkv, B_wo)
    return out[None]
```
